```python
import os as _os
_os.environ.setdefault("JAX_PLATFORMS", "cpu")
import jax
import jax.numpy as jnp

def _softmax(x, axis=-1):
    return jax.nn.softmax(x, axis=axis)
def _gelu(x):
    return jax.nn.gelu(x, approximate=True)
def _silu(x):
    return jax.nn.silu(x)
def _sigmoid(x):
    return jax.nn.sigmoid(x)
def _layernorm(x, axis=-1, eps=1e-5):
    m = jnp.mean(x, axis=axis, keepdims=True)
    v = jnp.var(x, axis=axis, keepdims=True)
    return (x - m) / jnp.sqrt(v + eps)
def _scatter_add(tgt, idx, src, axis=0):
    return tgt.at[idx].add(src)
def _segment_sum(src, seg, n):
    return jax.ops.segment_sum(src, seg, n)
class _Rng:
    def __init__(self, key):
        self._k = key
    def _next(self):
        self._k, sub = jax.random.split(self._k)
        return sub
    def normal(self, shape):
        return jax.random.normal(self._next(), shape, dtype=jnp.bfloat16)
    def randint(self, lo, hi, shape):
        return jax.random.randint(self._next(), shape, lo, hi, dtype=jnp.int32)
    def uniform(self, shape, lo=0.0, hi=1.0):
        return jax.random.uniform(self._next(), shape, jnp.bfloat16, lo, hi)
    def permutation(self, n):
        return jax.random.permutation(self._next(), n)


kernel_name = 'standalone__channel_attn_cbam__vision'

def setup_inputs():
    _rng = _Rng(jax.random.key(int.from_bytes(__import__("os").urandom(4), "little")))
    _w = (lambda a: (lambda t: t.astype(jnp.bfloat16) if jnp.issubdtype(t.dtype, jnp.floating) else t)(jnp.asarray(a)))
    H = W = 224
    C = 192
    r = max(C // 4, 1)
    return {
        "x": _w((lambda *s: _rng.normal(s) * 0.2)(1, H, W, C) + (lambda *s: _rng.normal(s) * 0.2)(1, 1, 1, C) * 2.0),
        "w1": _w((lambda *s: _rng.normal(s) * 0.2)(C, r)),
        "w2": _w((lambda *s: _rng.normal(s) * 0.2)(r, C)),
    }

def reference(x, w1, w2):
    B, H, W, C = x.shape
    xf = x.reshape(B, H * W, C)
    gap = jnp.mean(xf, 1)
    gmp = jnp.amax(xf, 1)
    h_a = gap @ w1
    h_a = h_a * (lambda x, dt: x.astype(dt))(h_a > 0, h_a.dtype)
    h_m = gmp @ w1
    h_m = h_m * (lambda x, dt: x.astype(dt))(h_m > 0, h_m.dtype)
    scale = _sigmoid(h_a @ w2 + h_m @ w2)
    return x * scale[:, None, None, :]
```

```python
import jax
import jax.numpy as jnp
from jax import lax
import jax.experimental.pallas as pl
import jax.experimental.pallas.tpu as pltpu

H = W = 224
C = 192
R = 48
LANES = 128
GROUPS = C // 8
COLS = 128
PHASES = 3
SLABS = H * GROUPS // (COLS * PHASES)
SHIFT = COLS % GROUPS

READ_COLS = 4
READ_TAIL = (2, 1, 1)
WRITE_COLS = 2
TAIL_START = COLS - sum(READ_TAIL)
N_READS = TAIL_START // READ_COLS


def _tree(op, xs):
    while len(xs) > 1:
        xs = [
            op(xs[i], xs[i + 1]) if i + 1 < len(xs) else xs[i]
            for i in range(0, len(xs), 2)
        ]
    return xs[0]


def _round_bf16(v):
    return v.astype(jnp.bfloat16).astype(jnp.float32)


def _rows(col, n):
    if isinstance(col, int):
        return pl.ds(col * 8, n * 8)
    return pl.ds(pl.multiple_of(col * 8, 8), n * 8)


def _group(col, r):
    if isinstance(col, int) and isinstance(r, int):
        return (SHIFT * r + col) % GROUPS
    return lax.rem(SHIFT * r + col, GROUPS)


def _kernel(
    x_hbm, w1t_hbm, w2_hbm, o_hbm,
    buf, w1t_v, w2_v, w1c, w2c, sum_acc, max_acc, scale,
    read_sems, write_sem, w_sem,
):
    f32 = jnp.float32

    def read(col, n, i):
        sl = (slice(None), slice(None), _rows(col, n), slice(None))
        return pltpu.make_async_copy(x_hbm.at[sl], buf.at[sl], read_sems.at[i])

    def write(col, n):
        sl = (slice(None), slice(None), _rows(col, n), slice(None))
        return pltpu.make_async_copy(buf.at[sl], o_hbm.at[sl], write_sem)

    def load(col, n, r):
        return [buf[a, r, _rows(col, n), :].astype(f32) for a in range(SLABS)]

    tail = [
        (TAIL_START + sum(READ_TAIL[:t]), n, N_READS + t)
        for t, n in enumerate(READ_TAIL)
    ]

    w1_copy = pltpu.make_async_copy(w1t_hbm, w1t_v, w_sem)
    w2_copy = pltpu.make_async_copy(w2_hbm, w2_v, w_sem)
    read(0, READ_COLS, 0).start()
    w1_copy.start()
    w2_copy.start()

    @pl.loop(1, N_READS)
    def _(i):
        read(i * READ_COLS, READ_COLS, i).start()

    for col, n, i in tail:
        read(col, n, i).start()

    sum_acc[...] = jnp.zeros(sum_acc.shape, f32)
    max_acc[...] = jnp.full(max_acc.shape, -jnp.inf, f32)

    w1_copy.wait()
    w2_copy.wait()
    for src, dst in ((w1t_v, w1c), (w2_v, w2c)):
        w = src[...].astype(f32)
        pad = jnp.zeros((LANES - 2 * R, C), f32)
        dst[...] = jnp.concatenate([w, w, pad], axis=0).T

    @pl.loop(0, N_READS)
    def _(i):
        col = i * READ_COLS
        read(col, READ_COLS, i).wait()

        @pl.loop(0, PHASES)
        def _(r):
            ch = _rows(_group(col, r), READ_COLS)
            vs = load(col, READ_COLS, r)
            s = m = vs[0]
            for v in vs[1:]:
                s = s + v
                m = jnp.maximum(m, v)
            sum_acc[ch, :] = sum_acc[ch, :] + s
            max_acc[ch, :] = jnp.maximum(max_acc[ch, :], m)

    def pool_and_project(group, n, vs):
        ch = _rows(group, n)
        s = _tree(jnp.add, [sum_acc[ch, :]] + vs)
        m = _tree(jnp.maximum, [max_acc[ch, :]] + vs)
        gap = _round_bf16(jnp.sum(s, axis=1, keepdims=True) / float(H * W))
        gmp = jnp.max(m, axis=1, keepdims=True)
        lane = lax.broadcasted_iota(jnp.int32, (8 * n, LANES), 1)
        p = w1c[ch, :] * jnp.where(lane < R, gap, gmp)
        return _tree(jnp.add, [p[8 * k:8 * k + 8] for k in range(n)])

    first_final = COLS - SHIFT
    h = _tree(jnp.add, [
        pool_and_project(_group(first_final, r), TAIL_START - first_final, [])
        for r in range(PHASES)
    ])
    for col, n, i in tail:
        read(col, n, i).wait()
        h = _tree(jnp.add, [h] + [
            pool_and_project(_group(col, r), n, load(col, n, r))
            for r in range(PHASES)
        ])
    lane = lax.broadcasted_iota(jnp.int32, (8, LANES), 1)
    h = jnp.where(lane < 2 * R, h, 0.0)
    h = _round_bf16(jnp.sum(h, axis=0, keepdims=True))
    h = jnp.broadcast_to(h * (h > 0).astype(f32), (8, LANES))

    def scale_in_place(col, n, r, s):
        s = jnp.concatenate([s, s[:, :W - LANES]], axis=1)
        for a in range(SLABS):
            idx = (a, r, _rows(col, n), slice(None))
            buf[idx] = (buf[idx].astype(f32) * s).astype(buf.dtype)

    @pl.loop(0, SHIFT)
    def _(col):
        ss = []
        for r in range(PHASES):
            ch = _rows(SHIFT * r + col, 1)
            z = _round_bf16(jnp.sum(w2c[ch, :] * h, axis=1, keepdims=True))
            s = jnp.broadcast_to(_round_bf16(jax.nn.sigmoid(z)), (8, LANES))
            scale[ch, :] = s
            ss.append(s)
        for r in range(PHASES):
            scale_in_place(col, 1, r, ss[r])
        write(col, 1).start()

    @pl.loop(0, (COLS - SHIFT) // WRITE_COLS)
    def _(i):
        col = SHIFT + i * WRITE_COLS

        @pl.loop(0, PHASES)
        def _(r):
            s = scale[_rows(_group(col, r), WRITE_COLS), :]
            scale_in_place(col, WRITE_COLS, r, s)

        write(col, WRITE_COLS).start()

    pltpu.make_async_copy(buf, o_hbm, write_sem).wait()


@jax.jit
def pallas_standalone__channel_attn_cbam__vision_kernel(
    x: jax.Array,
    w1: jax.Array,
    w2: jax.Array,
):
    assert x.shape == (1, H, W, C) and w1.shape == (C, R) and w2.shape == (R, C)
    view = (SLABS, PHASES, COLS * 8, W)
    hbm = pl.BlockSpec(memory_space=pltpu.HBM)
    out = pl.pallas_call(
        _kernel,
        out_shape=jax.ShapeDtypeStruct(view, x.dtype),
        in_specs=[hbm, hbm, hbm],
        out_specs=hbm,
        scratch_shapes=[
            pltpu.VMEM(view, x.dtype),
            pltpu.VMEM((R, C), w1.dtype),
            pltpu.VMEM((R, C), w2.dtype),
            pltpu.VMEM((C, LANES), jnp.float32),
            pltpu.VMEM((C, LANES), jnp.float32),
            pltpu.VMEM((C, W), jnp.float32),
            pltpu.VMEM((C, W), jnp.float32),
            pltpu.VMEM((C, LANES), jnp.float32),
            pltpu.SemaphoreType.DMA((N_READS + len(READ_TAIL),)),
            pltpu.SemaphoreType.DMA(()),
            pltpu.SemaphoreType.DMA(()),
        ],
        compiler_params=pltpu.CompilerParams(
            vmem_limit_bytes=64 * 1024 * 1024,
            disable_semaphore_checks=True,
        ),
    )(jnp.transpose(x, (0, 1, 3, 2)).reshape(view), w1.T, w2)
    return jnp.transpose(out.reshape(1, H, C, W), (0, 1, 3, 2))
```
